```python
import os as _os
_os.environ.setdefault("JAX_PLATFORMS", "cpu")
import jax
import jax.numpy as jnp

def _softmax(x, axis=-1):
    return jax.nn.softmax(x, axis=axis)
def _gelu(x):
    return jax.nn.gelu(x, approximate=True)
def _silu(x):
    return jax.nn.silu(x)
def _sigmoid(x):
    return jax.nn.sigmoid(x)
def _layernorm(x, axis=-1, eps=1e-5):
    m = jnp.mean(x, axis=axis, keepdims=True)
    v = jnp.var(x, axis=axis, keepdims=True)
    return (x - m) / jnp.sqrt(v + eps)
def _scatter_add(tgt, idx, src, axis=0):
    return tgt.at[idx].add(src)
def _segment_sum(src, seg, n):
    return jax.ops.segment_sum(src, seg, n)
class _Rng:
    def __init__(self, key):
        self._k = key
    def _next(self):
        self._k, sub = jax.random.split(self._k)
        return sub
    def normal(self, shape):
        return jax.random.normal(self._next(), shape, dtype=jnp.bfloat16)
    def randint(self, lo, hi, shape):
        return jax.random.randint(self._next(), shape, lo, hi, dtype=jnp.int32)
    def uniform(self, shape, lo=0.0, hi=1.0):
        return jax.random.uniform(self._next(), shape, jnp.bfloat16, lo, hi)
    def permutation(self, n):
        return jax.random.permutation(self._next(), n)


kernel_name = 'gated_mix__linear_attn_block__sliding_local_dilated__prompt'

def setup_inputs():
    _rng = _Rng(jax.random.key(int.from_bytes(__import__("os").urandom(4), "little")))
    _w = (lambda a: (lambda t: t.astype(jnp.bfloat16) if jnp.issubdtype(t.dtype, jnp.floating) else t)(jnp.asarray(a)))
    def _A_setup():
        B, S, D = 1, 2048, 512
        return {
            "x": _w((lambda *s: _rng.normal(s) * 0.05)(B, S, D)),
            "wqkv": _w((lambda *s: _rng.normal(s) * 1.6)(D, 3 * D)),
            "wo": _w((lambda *s: _rng.normal(s) * 0.8)(D, D)),
        }
    _A_in = _A_setup()

    def _B_setup():
        B, S, D = 1, 2048, 512
        return {
            "x": _w((lambda *s: _rng.normal(s) * 0.05)(B, S, D)),
            "wqkv": _w((lambda *s: _rng.normal(s) * 0.8)(D, 3 * D)),
            "wo": _w((lambda *s: _rng.normal(s) * 0.05)(D, D)),
        }
    _B_in = _B_setup()

    return {
        "A_x": _A_in["x"],
        "A_wqkv": _A_in["wqkv"],
        "A_wo": _A_in["wo"],
        "B_x": _B_in["x"],
        "B_wqkv": _B_in["wqkv"],
        "B_wo": _B_in["wo"],
        "gate_w": _w((lambda *s: _rng.normal(s) * 0.05)(512) * 16.0),
    }

def reference(A_x, A_wqkv, A_wo, B_x, B_wqkv, B_wo, gate_w):
    def _A_ref(x, wqkv, wo):
        B, S, D = x.shape
        H = 32; Dh = D // H
        qkv = (lambda x, *d: x.transpose(*d))((x @ wqkv).reshape(B, S, 3, H, Dh), 2, 0, 3, 1, 4)
        q, k, v = qkv[0], qkv[1], qkv[2]
        phi = lambda t: jnp.where(t > 0, t + 1, jnp.exp(t)) + 1e-6
        pq, pk = phi(q), phi(k)
        kv = jnp.einsum("bhsd,bhse->bhde", pk, v)
        z = jnp.einsum("bhsd->bhd", pk)
        num = jnp.einsum("bhqd,bhde->bhqe", pq, kv)
        den = jnp.einsum("bhqd,bhd->bhq", pq, z)[..., None] + 1e-6
        o = num / den
        return (lambda x, *d: x.transpose(*d))(o, 0, 2, 1, 3).reshape(B, S, D) @ wo

    def _B_ref(x, wqkv, wo):
        B, S, D = x.shape
        H = 32; Dh = D // H
        W, dil = 8, 2
        qkv = (lambda x, *d: x.transpose(*d))((x @ wqkv).reshape(B, S, 3, H, Dh), 2, 0, 3, 1, 4)
        q, k, v = qkv[0], qkv[1], qkv[2]
        scale = Dh ** -0.5
        pos = jnp.arange(S)
        off = jnp.arange(W) * dil
        idx = pos[:, None] - off[None, :]
        mask = idx >= 0
        idx_c = jnp.where(mask, idx, 0).reshape(-1)
        kg = k[:, :, idx_c, :].reshape(B, H, S, W, Dh)
        vg = v[:, :, idx_c, :].reshape(B, H, S, W, Dh)
        logits = jnp.einsum("bhsd,bhswd->bhsw", q, kg) * scale
        logits = jnp.where(mask[None, None, :, :], logits, -1e9)
        attn = _softmax(logits, axis=-1)
        o = jnp.einsum("bhsw,bhswd->bhsd", attn, vg)
        return (lambda x, *d: x.transpose(*d))(o, 0, 2, 1, 3).reshape(B, S, D) @ wo

    x = A_x
    g = _sigmoid((x * gate_w).sum(-1, keepdims=True))
    a = _A_ref(x, A_wqkv, A_wo)
    b = _B_ref(x, B_wqkv, B_wo)
    return g * a + (1 - g) * b
```

```python
import jax
import jax.numpy as jnp
import jax.experimental.pallas as pl
import jax.experimental.pallas.tpu as pltpu

S, D, H, DH, W, DIL = 2048, 512, 32, 16, 8, 2
T = 256
NT = S // T
PAD = 16
F32, BF16 = jnp.float32, jnp.bfloat16
LOG2E = 1.4426950408889634


def _phi(t):
    return jnp.where(t > 0, t + 1.0, jnp.exp(t)) + 1e-6


def _permute_cols(w_ref, c0, dst_ref, d0):
    R = 64
    lane = jax.lax.broadcasted_iota(jnp.int32, (R // 2, 128), 1)
    hh = lane & 31
    dd = lane >> 5
    src_tile = hh >> 3
    base = (hh & 7) * 16 + dd
    for r in range(0, D, R):
        tiles = [pltpu.bitcast(w_ref[r:r + R, c0 + 128 * j:c0 + 128 * (j + 1)], jnp.int32) for j in range(4)]
        for jp in range(4):
            idx = base + 4 * jp
            g = [jnp.take_along_axis(t, idx, axis=1) for t in tiles]
            o = jnp.where(src_tile == 0, g[0], jnp.where(src_tile == 1, g[1], jnp.where(src_tile == 2, g[2], g[3])))
            dst_ref[r:r + R, d0 + 128 * jp:d0 + 128 * (jp + 1)] = pltpu.bitcast(o, BF16)


def kernel(xa_ref, wa_ref, woa_ref, wb_ref, wob_ref, gw_ref, o_ref,
           wbp_ref, wcat_ref, g_ref, z_ref, zbd_ref, kb_ref, vb_ref, wof_ref):
    p = pl.program_id(0)
    j = pl.program_id(1)

    @pl.when((p == 0) & (j == 0))
    def _init():
        g_ref[...] = jnp.zeros_like(g_ref)
        z_ref[...] = jnp.zeros_like(z_ref)
        for c in range(4):
            kb_ref[c, 0:PAD, :] = jnp.zeros((PAD, 128), F32)
            vb_ref[c, 0:PAD, :] = jnp.zeros((PAD, 128), F32)
        for i in range(3):
            _permute_cols(wb_ref, i * D, wbp_ref, i * D)
        for c in range(4):
            wof_ref[c] = wob_ref[:, 128 * c:128 * (c + 1)].astype(F32)
        for c in range(4):
            for d in range(DH):
                wcat_ref[D + d * H:D + (d + 1) * H, 128 * c:128 * (c + 1)] = (
                    wof_ref[c, pl.ds(d, H, stride=DH), :].astype(BF16))

    @pl.when(p == 0)
    def _phase0():
        x = xa_ref[...]
        k = jnp.dot(x, wa_ref[:, D:2 * D], preferred_element_type=F32)
        pk = _phi(k)
        z_ref[...] += jnp.sum(pk.reshape(T // 8, 8, D), axis=0)
        g_ref[...] += jax.lax.dot_general(pk.astype(BF16), x, (((0,), (0,)), ((), ())),
                                          preferred_element_type=F32)

    @pl.when((p == 1) & (j == 0))
    def _mid():
        r = jax.lax.broadcasted_iota(jnp.int32, (128, 128), 0) >> 4
        c = jax.lax.broadcasted_iota(jnp.int32, (128, 128), 1) >> 4
        same = r == c
        z = jnp.sum(z_ref[...], axis=0, keepdims=True)
        for t in range(4):
            sl = slice(128 * t, 128 * (t + 1))
            kv = jnp.dot(g_ref[sl, :].astype(BF16), wa_ref[:, 2 * D + 128 * t:2 * D + 128 * (t + 1)],
                         preferred_element_type=F32)
            kv = jnp.where(same, kv, 0.0).astype(BF16)
            wcat_ref[sl, :] = jnp.dot(kv, woa_ref[sl, :], preferred_element_type=F32).astype(BF16)
            zt = jnp.broadcast_to(z[:, sl], (128, 128)).T
            zbd_ref[sl, :] = jnp.where(same, zt, 0.0).astype(BF16)

    @pl.when(p == 1)
    def _phase1():
        x = xa_ref[...]
        gate = jax.nn.sigmoid(jnp.sum(x.astype(F32) * gw_ref[...].astype(F32), axis=-1, keepdims=True))
        q = jnp.dot(x, wa_ref[:, 0:D], preferred_element_type=F32)
        pq = _phi(q)
        pqb = pq.astype(BF16)
        parts = []
        for t in range(4):
            sl = slice(128 * t, 128 * (t + 1))
            den = jnp.dot(pqb[:, sl], zbd_ref[sl, :], preferred_element_type=F32) + 1e-6
            parts.append((pq[:, sl] * (gate / den)).astype(BF16))
        xb = x
        r0 = pl.multiple_of(j * T, T)
        qb = jnp.dot(xb, wbp_ref[:, 0:D], preferred_element_type=F32) * (DH ** -0.5 * LOG2E)
        kb = jnp.dot(xb, wbp_ref[:, D:2 * D], preferred_element_type=F32)
        vb = jnp.dot(xb, wbp_ref[:, 2 * D:3 * D], preferred_element_type=F32)
        for c in range(4):
            kb_ref[c, pl.ds(r0 + PAD, T), :] = kb[:, 128 * c:128 * (c + 1)]
            vb_ref[c, pl.ds(r0 + PAD, T), :] = vb[:, 128 * c:128 * (c + 1)]
        row = jax.lax.broadcasted_iota(jnp.int32, (T, 128), 0) + j * T
        logits = []
        for w in range(W):
            acc = None
            for c in range(4):
                t = qb[:, 128 * c:128 * (c + 1)] * kb_ref[c, pl.ds(r0 + PAD - DIL * w, T), :]
                acc = t if acc is None else acc + t
            acc = acc + pltpu.roll(acc, 64, 1)
            acc = acc + pltpu.roll(acc, 32, 1)
            if w > 0:
                acc = jnp.where(row >= DIL * w, acc, -1e9 * LOG2E)
            logits.append(acc)
        m = logits[0]
        for w in range(1, W):
            m = jnp.maximum(m, logits[w])
        e = [jnp.exp2(l - m) for l in logits]
        ssum = e[0]
        for w in range(1, W):
            ssum = ssum + e[w]
        inv = (1.0 - gate) / ssum
        for c in range(4):
            acc = None
            for w in range(W):
                t = e[w] * vb_ref[c, pl.ds(r0 + PAD - DIL * w, T), :]
                acc = t if acc is None else acc + t
            parts.append((acc * inv).astype(BF16))
        lhs = jnp.concatenate(parts, axis=1)
        o_ref[...] = jnp.dot(lhs, wcat_ref[...], preferred_element_type=F32).astype(o_ref.dtype)


@jax.jit
def pallas_gated_mix__linear_attn_block__sliding_local_dilated__prompt_kernel(
        A_x, A_wqkv, A_wo, B_x, B_wqkv, B_wo, gate_w):
    full = lambda shape: pl.BlockSpec(shape, lambda p, j: (0,) * len(shape))
    out = pl.pallas_call(
        kernel,
        grid=(2, NT),
        in_specs=[
            pl.BlockSpec((T, D), lambda p, j: (j, 0)),
            full((D, 3 * D)), full((D, D)), full((D, 3 * D)), full((D, D)), full((1, D)),
        ],
        out_specs=pl.BlockSpec((T, D), lambda p, j: (j * p, 0)),
        out_shape=jax.ShapeDtypeStruct((S, D), BF16),
        scratch_shapes=[
            pltpu.VMEM((D, 3 * D), BF16),
            pltpu.VMEM((2 * D, D), BF16),
            pltpu.VMEM((D, D), F32),
            pltpu.VMEM((8, D), F32),
            pltpu.VMEM((D, 128), BF16),
            pltpu.VMEM((4, S + PAD, 128), F32),
            pltpu.VMEM((4, S + PAD, 128), F32),
            pltpu.VMEM((4, D, 128), F32),
        ],
        compiler_params=pltpu.CompilerParams(
            dimension_semantics=("arbitrary", "arbitrary"),
            vmem_limit_bytes=100 * 1024 * 1024),
    )(A_x.reshape(S, D), A_wqkv, A_wo, B_wqkv, B_wo, gate_w.reshape(1, D))
    return out.reshape(1, S, D)
```

```python
import jax
import jax.numpy as jnp
import jax.experimental.pallas as pl
import jax.experimental.pallas.tpu as pltpu

S, D, H, DH, W, DIL = 2048, 512, 32, 16, 8, 2
T = 256
NT = S // T
PAD = 16
RC = 16
PR = 2 * D // NT
DPS = 2 * DH // NT
F32, BF16 = jnp.float32, jnp.bfloat16
LOG2E = 1.4426950408889634


def _phi(t):
    return jnp.where(t > 0, t + 1.0, jnp.exp(t)) + 1e-6


def _dot(a, b):
    return jnp.dot(a, b, preferred_element_type=F32)


def kernel(x_hbm, wa_hbm, woa_hbm, wb_hbm, wob_hbm, gw_ref, o_ref,
           xs, wa, woa, wb, wob, wbp, wcat, g_ref, z_ref, zbd, qb_ref, kb_ref, vb_ref, wof, lhs_ref, gate_ref,
           xsem, wsem):
    step = pl.program_id(0)

    def x_copy(i):
        return pltpu.make_async_copy(x_hbm.at[pl.ds(i * T, T)], xs.at[pl.ds(i * T, T)], xsem.at[i])
    wk_copy = pltpu.make_async_copy(wa_hbm.at[:, D:2 * D], wa.at[:, D:2 * D], wsem.at[0])
    wb_copy = pltpu.make_async_copy(wb_hbm, wb, wsem.at[1])
    wob_copy = pltpu.make_async_copy(wob_hbm, wob, wsem.at[2])
    wq_copy = pltpu.make_async_copy(wa_hbm.at[:, 0:D], wa.at[:, 0:D], wsem.at[3])
    wv_copy = pltpu.make_async_copy(wa_hbm.at[:, 2 * D:3 * D], wa.at[:, 2 * D:3 * D], wsem.at[4])
    woa_copy = pltpu.make_async_copy(woa_hbm, woa, wsem.at[5])

    @pl.when(step == 0)
    def _init():
        wk_copy.start()
        x_copy(0).start()
        wb_copy.start()
        x_copy(1).start()
        wob_copy.start()
        for i in range(2, NT):
            x_copy(i).start()
        wv_copy.start()
        woa_copy.start()
        wq_copy.start()
        g_ref[...] = jnp.zeros_like(g_ref)
        z_ref[...] = jnp.zeros_like(z_ref)
        for c in range(4):
            kb_ref[c, 0:PAD, :] = jnp.zeros((PAD, 128), F32)
            vb_ref[c, 0:PAD, :] = jnp.zeros((PAD, 128), F32)
        wk_copy.wait()

    @pl.when(step == NT // 2)
    def _():
        wb_copy.wait()
        wob_copy.wait()
        for c in range(4):
            wof[c] = wob[:, 128 * c:128 * (c + 1)].astype(F32)

    def phase0(with_perm):
        j = step
        x_copy(j).wait()
        r0 = pl.multiple_of(j * T, T)
        x = xs[pl.ds(r0, T), :]
        k = _dot(x, wa[:, D:2 * D])
        gw = gw_ref[...].astype(F32).reshape(1, D)
        gate_ref[pl.ds(r0, T), :] = jnp.broadcast_to(
            jax.nn.sigmoid(jnp.sum(x.astype(F32) * gw, axis=-1, keepdims=True)), (T, 128))
        pk = _phi(k)
        z_ref[...] += jnp.sum(pk.reshape(T // 8, 8, D), axis=0)
        g_ref[...] += jax.lax.dot_general(pk.astype(BF16), x, (((0,), (0,)), ((), ())),
                                          preferred_element_type=F32)
        if not with_perm:
            return
        j = step - NT // 2
        w0 = pl.multiple_of(j * PR, PR)
        lane = jax.lax.broadcasted_iota(jnp.int32, (PR // 2, 128), 1)
        hh = lane & 31
        src_tile = hh >> 3
        base = (hh & 7) * 16 + (lane >> 5)
        for i in range(3):
            tiles = [pltpu.bitcast(wb[pl.ds(w0, PR), i * D + 128 * s:i * D + 128 * (s + 1)], jnp.int32)
                     for s in range(4)]
            for jp in range(4):
                g = [jnp.take_along_axis(t, base + 4 * jp, axis=1) for t in tiles]
                o = jnp.where(src_tile == 0, g[0],
                              jnp.where(src_tile == 1, g[1], jnp.where(src_tile == 2, g[2], g[3])))
                wbp[pl.ds(w0, PR), i * D + 128 * jp:i * D + 128 * (jp + 1)] = pltpu.bitcast(o, BF16)
        for dd in range(DPS):
            d = j * DPS + dd
            for c in range(4):
                wcat[pl.ds(pl.multiple_of(D + d * H, H), H), 128 * c:128 * (c + 1)] = (
                    wof[c, pl.ds(d, H, stride=DH), :].astype(BF16))

    @pl.when(step < NT // 2)
    def _():
        phase0(False)

    @pl.when((step >= NT // 2) & (step < NT))
    def _():
        phase0(True)

    def qkv_b(i):
        r0 = pl.multiple_of(i * T, T)
        x = xs[pl.ds(r0, T), :]
        qb_ref[i % 2] = _dot(x, wbp[:, 0:D]) * (DH ** -0.5 * LOG2E)
        kb = _dot(x, wbp[:, D:2 * D])
        vb = _dot(x, wbp[:, 2 * D:3 * D])
        for c in range(4):
            kb_ref[c, pl.ds(r0 + PAD, T), :] = kb[:, 128 * c:128 * (c + 1)]
            vb_ref[c, pl.ds(r0 + PAD, T), :] = vb[:, 128 * c:128 * (c + 1)]

    @pl.when(step == NT)
    def _mid():
        wv_copy.wait()
        woa_copy.wait()
        wq_copy.wait()
        r = jax.lax.broadcasted_iota(jnp.int32, (128, 128), 0) >> 4
        c = jax.lax.broadcasted_iota(jnp.int32, (128, 128), 1) >> 4
        same = r == c
        z = jnp.sum(z_ref[...], axis=0, keepdims=True)
        for t in range(4):
            sl = slice(128 * t, 128 * (t + 1))
            kv = _dot(g_ref[sl, :].astype(BF16), wa[:, 2 * D + 128 * t:2 * D + 128 * (t + 1)])
            kv = jnp.where(same, kv, 0.0).astype(BF16)
            wcat[sl, :] = _dot(kv, woa[sl, :]).astype(BF16)
            zt = jnp.broadcast_to(z[:, sl], (128, 128)).T
            zbd[sl, :] = jnp.where(same, zt, 0.0).astype(BF16)
        qkv_b(0)

    def final(i):
        o_ref[...] = _dot(lhs_ref[i % 2], wcat[...]).astype(o_ref.dtype)

    def phase1(with_next, with_final):
        j = step - NT
        r0 = pl.multiple_of(j * T, T)
        x = xs[pl.ds(r0, T), :]
        gate = gate_ref[pl.ds(r0, T), :]
        th = []
        NW = 256
        pqs = {}

        def qa_piece(n):
            pq = _phi(_dot(x, wa[:, n:n + NW]))
            pqs[n] = pq

        def den_piece(n):
            pq = pqs[n]
            pqb = pq.astype(BF16)
            for t in range(0, NW, 128):
                den = _dot(pqb[:, t:t + 128], zbd[n + t:n + t + 128, :]) + 1e-6
                lhs_ref[j % 2, :, n + t:n + t + 128] = (pq[:, t:t + 128] * (gate / den)).astype(BF16)

        def fin_piece(n):
            o_ref[:, n:n + NW] = _dot(lhs_ref[(j - 1) % 2], wcat[:, n:n + NW]).astype(o_ref.dtype)

        def qkv_piece(n):
            r1 = pl.multiple_of((j + 1) * T, T)
            y = _dot(xs[pl.ds(r1, T), :], wbp[:, n:n + NW])
            if n < D:
                qb_ref[(j + 1) % 2, :, n:n + NW] = y * (DH ** -0.5 * LOG2E)
            else:
                dst = kb_ref if n < 2 * D else vb_ref
                for t in range(0, NW, 128):
                    dst[((n + t) % D) // 128, pl.ds(r1 + PAD, T), :] = y[:, t:t + 128]

        th += [(qa_piece, n) for n in range(0, D, NW)]
        if with_next:
            th += [(qkv_piece, n) for n in range(0, 3 * D, NW)]
        if with_final:
            th += [(fin_piece, n) for n in range(0, D, NW)]
        th += [(den_piece, n) for n in range(0, D, NW)]
        nch = T // RC
        sched = [[] for _ in range(nch)]
        for i, tk in enumerate(th):
            sched[i * nch // len(th)].append(tk)
        slot = j % 2
        for rc in range(0, T, RC):
            for f, n in sched[rc // RC]:
                f(n)
            row = jax.lax.broadcasted_iota(jnp.int32, (RC, 128), 0) + (j * T + rc)
            qs = [qb_ref[slot, rc:rc + RC, 128 * c:128 * (c + 1)] for c in range(4)]
            logits = []
            for w in range(W):
                acc = None
                for c in range(4):
                    t = qs[c] * kb_ref[c, pl.ds(r0 + rc + PAD - DIL * w, RC), :]
                    acc = t if acc is None else acc + t
                acc = acc + pltpu.roll(acc, 64, 1)
                acc = acc + pltpu.roll(acc, 32, 1)
                if w > 0 and rc < PAD:
                    acc = jnp.where(row >= DIL * w, acc, -1e9 * LOG2E)
                logits.append(acc)
            m = logits[0]
            for w in range(1, W):
                m = jnp.maximum(m, logits[w])
            e = [jnp.exp2(l - m) for l in logits]
            ssum = e[0]
            for w in range(1, W):
                ssum = ssum + e[w]
            inv = (1.0 - gate[rc:rc + RC]) / ssum
            for c in range(4):
                acc = None
                for w in range(W):
                    t = e[w] * vb_ref[c, pl.ds(r0 + rc + PAD - DIL * w, RC), :]
                    acc = t if acc is None else acc + t
                lhs_ref[slot, rc:rc + RC, D + 128 * c:D + 128 * (c + 1)] = (acc * inv).astype(BF16)

    @pl.when(step == NT)
    def _():
        phase1(True, False)

    @pl.when((step > NT) & (step < 2 * NT - 1))
    def _():
        phase1(True, True)

    @pl.when(step == 2 * NT - 1)
    def _():
        phase1(False, True)

    @pl.when(step == 2 * NT)
    def _():
        final(NT - 1)


@jax.jit
def pallas_gated_mix__linear_attn_block__sliding_local_dilated__prompt_kernel(
        A_x, A_wqkv, A_wo, B_x, B_wqkv, B_wo, gate_w):
    hbm = pl.BlockSpec(memory_space=pl.ANY)
    out = pl.pallas_call(
        kernel,
        grid=(2 * NT + 1,),
        in_specs=[hbm, hbm, hbm, hbm, hbm, pl.BlockSpec((D,), lambda i: (0,))],
        out_specs=pl.BlockSpec((T, D), lambda i: (jnp.maximum(i - NT - 1, 0), 0)),
        out_shape=jax.ShapeDtypeStruct((S, D), BF16),
        scratch_shapes=[
            pltpu.VMEM((S, D), BF16),
            pltpu.VMEM((D, 3 * D), BF16),
            pltpu.VMEM((D, D), BF16),
            pltpu.VMEM((D, 3 * D), BF16),
            pltpu.VMEM((D, D), BF16),
            pltpu.VMEM((D, 3 * D), BF16),
            pltpu.VMEM((2 * D, D), BF16),
            pltpu.VMEM((D, D), F32),
            pltpu.VMEM((8, D), F32),
            pltpu.VMEM((D, 128), BF16),
            pltpu.VMEM((2, T, D), F32),
            pltpu.VMEM((4, S + PAD, 128), F32),
            pltpu.VMEM((4, S + PAD, 128), F32),
            pltpu.VMEM((4, D, 128), F32),
            pltpu.VMEM((2, T, 2 * D), BF16),
            pltpu.VMEM((S, 128), F32),
            pltpu.SemaphoreType.DMA((NT,)),
            pltpu.SemaphoreType.DMA((6,)),
        ],
        compiler_params=pltpu.CompilerParams(
            dimension_semantics=("arbitrary",),
            vmem_limit_bytes=100 * 1024 * 1024),
    )(A_x.reshape(S, D), A_wqkv, A_wo, B_wqkv, B_wo, gate_w)
    return out.reshape(1, S, D)
```
